```python
import os as _os
_os.environ.setdefault('JAX_PLATFORMS', 'cpu')
import jax
import jax.numpy as jnp

def _softmax(x, axis=-1):
    return jax.nn.softmax(x, axis=axis)

def _gelu(x):
    return jax.nn.gelu(x, approximate=True)

def _silu(x):
    return jax.nn.silu(x)

def _sigmoid(x):
    return jax.nn.sigmoid(x)

def _layernorm(x, axis=-1, eps=1e-05):
    m = jnp.mean(x, axis=axis, keepdims=True)
    v = jnp.var(x, axis=axis, keepdims=True)
    return (x - m) / jnp.sqrt(v + eps)

def _scatter_add(tgt, idx, src, axis=0):
    return tgt.at[idx].add(src)

def _segment_sum(src, seg, n):
    return jax.ops.segment_sum(src, seg, n)

class _Rng:

    def __init__(self, key):
        self._k = key

    def _next(self):
        self._k, sub = jax.random.split(self._k)
        return sub

    def normal(self, shape):
        return jax.random.normal(self._next(), shape, dtype=jnp.bfloat16)

    def randint(self, lo, hi, shape):
        return jax.random.randint(self._next(), shape, lo, hi, dtype=jnp.int32)

    def uniform(self, shape, lo=0.0, hi=1.0):
        return jax.random.uniform(self._next(), shape, jnp.bfloat16, lo, hi)

    def permutation(self, n):
        return jax.random.permutation(self._next(), n)
kernel_name = 'adaLN_cond__sliding_local_dilated__mixer_channel_mlp__prompt'

def setup_inputs():
    _rng = _Rng(jax.random.key(int.from_bytes(__import__("os").urandom(4), "little")))
    _w = lambda a: (lambda t: t.astype(jnp.bfloat16) if jnp.issubdtype(t.dtype, jnp.floating) else t)(jnp.asarray(a))

    def _A_setup():
        B, S, D = (1, 2048, 512)
        return {'x': _w((lambda *s: _rng.normal(s) * 0.05)(B, S, D)), 'wqkv': _w((lambda *s: _rng.normal(s) * 0.05)(D, 3 * D)), 'wo': _w((lambda *s: _rng.normal(s) * 0.05)(D, D))}
    _A_in = _A_setup()

    def _B_setup():
        B, S, D, F = (1, 2048, 512, 1792)
        return {'x': _w((lambda *s: _rng.normal(s) * 0.05)(B, S, D)), 'w1': _w((lambda *s: _rng.normal(s) * 0.8)(D, F) * D ** (-0.5)), 'b1': _w((lambda *s: _rng.normal(s) * 0.8)(F)), 'w2': _w((lambda *s: _rng.normal(s) * 0.8)(F, D) * F ** (-0.5)), 'b2': _w((lambda *s: _rng.normal(s) * 0.4)(D))}
    _B_in = _B_setup()
    return {'A_x': _A_in['x'], 'A_wqkv': _A_in['wqkv'], 'A_wo': _A_in['wo'], 'B_x': _B_in['x'], 'B_w1': _B_in['w1'], 'B_b1': _B_in['b1'], 'B_w2': _B_in['w2'], 'B_b2': _B_in['b2'], 'c': _w((lambda *s: _rng.normal(s) * 0.05)(1, 512) * 8.0), 'w_mod': _w((lambda *s: _rng.normal(s) * 0.05)(512, 6 * 512) * 512 ** (-0.5) * 8.0)}

def reference(A_x, A_wqkv, A_wo, B_x, B_w1, B_b1, B_w2, B_b2, c, w_mod):

    def _A_ref(x, wqkv, wo):
        B, S, D = x.shape
        H = 32
        Dh = D // H
        W, dil = (8, 2)
        qkv = (lambda x, *d: x.transpose(*d))((x @ wqkv).reshape(B, S, 3, H, Dh), 2, 0, 3, 1, 4)
        q, k, v = (qkv[0], qkv[1], qkv[2])
        scale = Dh ** (-0.5)
        pos = jnp.arange(S)
        off = jnp.arange(W) * dil
        idx = pos[:, None] - off[None, :]
        mask = idx >= 0
        idx_c = jnp.where(mask, idx, 0).reshape(-1)
        kg = k[:, :, idx_c, :].reshape(B, H, S, W, Dh)
        vg = v[:, :, idx_c, :].reshape(B, H, S, W, Dh)
        logits = jnp.einsum('bhsd,bhswd->bhsw', q, kg) * scale
        logits = jnp.where(mask[None, None, :, :], logits, -1000000000.0)
        attn = _softmax(logits, axis=-1)
        o = jnp.einsum('bhsw,bhswd->bhsd', attn, vg)
        return (lambda x, *d: x.transpose(*d))(o, 0, 2, 1, 3).reshape(B, S, D) @ wo

    def _B_ref(x, w1, b1, w2, b2):
        y = _layernorm(x, axis=-1)
        h = _gelu(jnp.einsum('bsd,df->bsf', y, w1) + b1)
        return jnp.einsum('bsf,fd->bsd', h, w2) + b2
    x = A_x
    mod = (_silu(c) @ w_mod).reshape(c.shape[0], 6, 1, -1)
    sa, ca, ga, sb, cb, gb = (mod[:, 0].copy(), mod[:, 1].copy(), mod[:, 2].copy(), mod[:, 3].copy(), mod[:, 4].copy(), mod[:, 5].copy())
    h = _layernorm(x, axis=-1) * (1 + ca) + sa
    x = x + ga * _A_ref(h, A_wqkv, A_wo)
    h = _layernorm(x, axis=-1) * (1 + cb) + sb
    x = x + gb * _B_ref(h, B_w1, B_b1, B_w2, B_b2)
    return x
```

```python
import functools
import jax
import jax.numpy as jnp
from jax import lax
import jax.experimental.pallas as pl
import jax.experimental.pallas.tpu as pltpu

F32 = jnp.float32
BF16 = jnp.bfloat16
U32 = jnp.uint32
I32 = jnp.int32
H = 32
DH = 16
W = 8
DIL = 2
HALO = 16
EPS = 1e-5
LOG2E = 1.4426950408889634
GC0 = 0.7978845608028654
GC1 = GC0 * 0.044715
GS = GC1 ** (1.0 / 3.0)
GK = GC0 / GS


def _center(x):
    inv = 1.0 / x.shape[-1]
    m = jnp.sum(x, axis=-1, keepdims=True) * inv
    xc = x - m
    v = jnp.sum(xc * xc, axis=-1, keepdims=True) * inv
    return xc, lax.rsqrt(v + EPS)


def make_kernel(TM=256, RC=16, FCS=(256,) * 7, ASTART=0.0, ASTOP=0.95, SPLIT=1, NTOK=4,
                LC=32, L2START=0.0, L2STOP=0.8, L1START=0.0, L1STOP=0.8, WSPLIT=4, VAR1=0,
                PACE_L2=1, PACE_L1=1):
    def kernel(x_hbm, wqkv_hbm, wo_hbm, w1_hbm, b1_hbm, w2_hbm, b2_hbm, c_hbm, wmod_hbm,
               o_ref,
               x_s, wqkv_v, wo_v, w1_v, b1_v, w2_v, b2_v, c_v, wmod_v,
               mod_s, b1_s, wqkv_p, wo_f, wo_p, qkv_s, o_s, a_s, h_s, z_s, wsem):
        i = pl.program_id(0)
        NT = pl.num_programs(0) - 1
        S, D = x_hbm.shape
        F = w1_hbm.shape[-1]
        NB = D // 128
        QO, KO, VO = 0, NB, 2 * NB
        fcs = []
        f0 = 0
        for fc in FCS:
            fcs.append((f0, fc))
            f0 += fc
        assert f0 == F
        fsplit = fcs[WSPLIT][0]

        def xcopy(t):
            r = pl.multiple_of(t * TM, TM)
            return pltpu.make_async_copy(x_hbm.at[pl.ds(r, TM), :], x_s.at[pl.ds(r, TM), :], wsem.at[13 + t])

        cp = {}
        def defcopy(name, src, dst):
            cp[name] = pltpu.make_async_copy(src, dst, wsem.at[len(cp)])
        defcopy('c', c_hbm, c_v)
        defcopy('b1', b1_hbm, b1_v)
        defcopy('b2', b2_hbm, b2_v)
        for p, n in enumerate(('wq', 'wk', 'wv')):
            defcopy(n, wqkv_hbm.at[:, p * D:(p + 1) * D], wqkv_v.at[:, p * D:(p + 1) * D])
        defcopy('wma', wmod_hbm.at[:, 0:2 * D], wmod_v.at[:, 0:2 * D])
        defcopy('wmb', wmod_hbm.at[:, 2 * D:6 * D], wmod_v.at[:, 2 * D:6 * D])
        defcopy('wo', wo_hbm, wo_v)
        defcopy('w1a', w1_hbm.at[:, 0:fsplit], w1_v.at[:, 0:fsplit])
        defcopy('w2a', w2_hbm.at[0:fsplit, :], w2_v.at[0:fsplit, :])
        defcopy('w1b', w1_hbm.at[:, fsplit:F], w1_v.at[:, fsplit:F])
        defcopy('w2b', w2_hbm.at[fsplit:F, :], w2_v.at[fsplit:F, :])

        def modv(k):
            return mod_s[k]

        def bc(v8, rows):
            return jnp.broadcast_to(v8[0:1, :], (rows, v8.shape[-1]))

        def zero():
            return z_s[0]

        def fence_qkv(tok):
            row = pl.multiple_of(HALO + TM + 8 * zero(), 8)
            qkv_s[0, pl.ds(row, 8), :] = tok

        def fence_a(tok):
            row = pl.multiple_of(TM + 8 * zero(), 8)
            a_s[pl.ds(row, 8), 0:128] = tok

        def fence_x(tok):
            row = pl.multiple_of(S + 16 * zero(), 16)
            x_s[pl.ds(row, 16), 0:128] = jnp.concatenate([tok, tok], axis=0).astype(BF16)

        def pick(toks, n, lo, hi):
            nt = len(toks)
            return [toks[min(nt - 1, int(lo * nt + (u * (hi - lo) * nt) / n))] for u in range(n)]

        def silu8():
            c = c_v[...].astype(F32)
            s = c * jax.nn.sigmoid(c)
            return jnp.broadcast_to(s, (8, D)).astype(BF16)

        def perm_consts():
            lane = lax.broadcasted_iota(I32, (D // 2, 128), 1)
            b = (lane >> 2) & 3
            src = lax.broadcasted_iota(I32, (128, 128), 0)
            dst = lax.broadcasted_iota(I32, (128, 128), 1)
            ps = []
            for j in range(NB):
                ii = (j + ((src >> 2) & 3)) & 3
                tgt = (src & 3) * 32 + ii * 8 + (src >> 4)
                ps.append(jnp.where(dst == tgt, 1.0, 0.0).astype(BF16))
            return b, ps

        def perm_cols(p, b, ps):
            blk = [pltpu.bitcast(wqkv_v[:, p * D + k * 128:p * D + (k + 1) * 128], U32) for k in range(NB)]
            for j in range(NB):
                m = jnp.where(b == 0, blk[j], blk[(j + 1) % NB])
                m = jnp.where(b == 2, blk[(j + 2) % NB], m)
                m = jnp.where(b == 3, blk[(j + 3) % NB], m)
                t = jnp.dot(pltpu.bitcast(m, BF16), ps[j], preferred_element_type=F32)
                wqkv_p[:, p * D + j * 128:p * D + (j + 1) * 128] = pltpu.bitcast(t.astype(BF16), U32)

        def perm_wo():
            for k in range(NB):
                wo_f[k] = wo_v[:, k * 128:(k + 1) * 128].astype(F32)
            for j in range(NB):
                for e in range(4):
                    for k in range(NB):
                        rows = []
                        for ii in range(4):
                            g = (ii - j) % 4
                            rows.append(wo_f[k, pl.ds(ii * 128 + g * 4 + e, 8, stride=DH), :])
                        v = jnp.concatenate(rows, axis=0).astype(BF16)
                        r = (j * 128 + e * 32) // 2
                        wo_p[r:r + 16, k * 128:(k + 1) * 128] = pltpu.bitcast(v, U32)

        def l1(t, r0, n):
            row = pl.multiple_of(t * TM + r0, 16)
            x = x_s[pl.ds(row, n), :].astype(F32)
            xc, rs = _center(x)
            h = (xc * rs) * bc(modv(1), n) + bc(modv(0), n)
            h_s[r0 // 2:(r0 + n) // 2, :] = pltpu.bitcast(h.astype(BF16), U32)

        def halo():
            qkv_s[KO:, 0:HALO, :] = qkv_s[KO:, TM:TM + HALO, :]

        def qkv_part(p):
            h = pltpu.bitcast(h_s[...], BF16)
            r = jnp.dot(h, pltpu.bitcast(wqkv_p[:, p * D:(p + 1) * D], BF16), preferred_element_type=F32)
            if p == 0:
                r = r * ((DH ** -0.5) * LOG2E)
            for j in range(NB):
                qkv_s[p * NB + j, HALO:HALO + TM, :] = r[:, j * 128:(j + 1) * 128]
            hm = TM // NTOK
            return [r[k:k + 8, c:c + 128] for c in range(0, D, 128) for k in range(0, TM, hm)]

        def a_qk(r0, first):
            q = [qkv_s[QO + j, HALO + r0:HALO + r0 + RC, :] for j in range(NB)]
            lg = []
            for w in range(W):
                st = HALO + r0 - DIL * w
                acc = q[0] * qkv_s[KO, st:st + RC, :]
                for j in range(1, NB):
                    acc = acc + q[j] * qkv_s[KO + j, st:st + RC, :]
                acc = acc + pltpu.roll(acc, 64, 1)
                acc = acc + pltpu.roll(acc, 32, 1)
                if first and r0 < HALO and w > 0:
                    row = r0 + lax.broadcasted_iota(I32, (RC, 128), 0)
                    acc = jnp.where(row >= DIL * w, acc, -1e9 * LOG2E)
                lg.append(acc)
            m = lg[0]
            for w in range(1, W):
                m = jnp.maximum(m, lg[w])
            p = [jnp.exp2(l - m) for l in lg]
            den = p[0]
            for w in range(1, W):
                den = den + p[w]
            return p, pl.reciprocal(den, approx=True)

        def a_pv(r0, p, rden):
            for j in range(NB):
                st = HALO + r0
                acc = p[0] * qkv_s[VO + j, st:st + RC, :]
                for w in range(1, W):
                    st = HALO + r0 - DIL * w
                    acc = acc + p[w] * qkv_s[VO + j, st:st + RC, :]
                o_s[r0 // 2:(r0 + RC) // 2, j * 128:(j + 1) * 128] = pltpu.bitcast((acc * rden).astype(BF16), U32)

        def wo_mm():
            a = jnp.dot(pltpu.bitcast(o_s[...], BF16), pltpu.bitcast(wo_p[...], BF16), preferred_element_type=F32)
            a_s[0:TM, :] = a
            hm = TM // NTOK
            return [a[k:k + 8, c:c + 128] for c in range(0, D, 128) for k in range(0, TM, hm)]

        def l2(t, r0, n):
            row = pl.multiple_of(t * TM + r0, 16)
            x1 = x_s[pl.ds(row, n), :].astype(F32) + bc(modv(2), n) * a_s[r0:r0 + n, :]
            xc, rs = _center(x1)
            h2 = (xc * rs) * bc(modv(4), n) + bc(modv(3), n)
            hc, rs2 = _center(h2)
            y = (hc * (rs2 * GS)).astype(BF16)
            return x1 + bc(modv(6), n), y

        def mlp(y, f0, fc):
            n = y.shape[0]
            z = jnp.dot(y, w1_v[:, f0:f0 + fc], preferred_element_type=F32) + bc(b1_s[:, f0:f0 + fc], n)
            g = (z + z * jnp.tanh(z * (z * z + GK))).astype(BF16)
            part = jnp.dot(g, w2_v[f0:f0 + fc, :], preferred_element_type=F32)
            hm = n // NTOK
            toks = [z[r:r + 8, c:c + 128] for c in range(0, fc, 128) for r in range(0, n, hm)]
            toks += [part[r:r + 8, c:c + 128] for c in range(0, D, min(D, 65536 // fc)) for r in range(0, n, hm)]
            return part, toks

        def wait_w(name, always):
            if always:
                cp[name].wait()
            else:
                @pl.when(i == 1)
                def _():
                    cp[name].wait()

        def mlp_all(y, waits):
            acc = None
            toks = []
            for n, (f0, fc) in enumerate(fcs):
                if waits is not None and n == 0:
                    wait_w('w1a', waits); wait_w('w2a', waits)
                if waits is not None and n == WSPLIT:
                    wait_w('w1b', waits); wait_w('w2b', waits)
                part, tk = mlp(y, f0, fc)
                toks += tk
                acc = part if acc is None else acc + part
            return acc, toks

        def out(x1b, acc):
            o_ref[...] = (x1b + bc(modv(5), TM) * acc).astype(o_ref.dtype)

        rcs = list(range(0, TM, RC))
        lcs = list(range(0, TM, LC))

        @pl.when(i == 0)
        def _():
            z_s[0] = 0
            xcopy(0).start()
            for n in ('c', 'wq', 'wma', 'wk', 'wv', 'b1', 'b2', 'wo'):
                cp[n].start()
            xcopy(1).start()
            cp['wmb'].start()
            xcopy(2).start()
            for n in ('w1a', 'w2a', 'w1b', 'w2b'):
                cp[n].start()
            b, ps = perm_consts()
            qkv_s[KO:, 0:HALO, :] = jnp.zeros((2 * NB, HALO, 128), F32)
            cp['wq'].wait()
            perm_cols(0, b, ps)
            cp['c'].wait()
            s8 = silu8()
            cp['wma'].wait()
            ma = jnp.dot(s8, wmod_v[:, 0:2 * D], preferred_element_type=F32)
            mod_s[0] = ma[:, 0:D]
            mod_s[1] = 1.0 + ma[:, D:2 * D]
            xcopy(0).wait()
            for r0 in lcs:
                l1(0, r0, LC)
            qkv_part(0)
            cp['wk'].wait()
            perm_cols(1, b, ps)
            qkv_part(1)
            cp['wv'].wait()
            perm_cols(2, b, ps)
            qkv_part(2)
            cp['wo'].wait()
            perm_wo()
            for r0 in rcs:
                p, rden = a_qk(r0, True)
                a_pv(r0, p, rden)
            wo_mm()
            xcopy(1).wait()
            for r0 in lcs:
                l1(1, r0, LC)
            cp['b1'].wait()
            cp['b2'].wait()
            cp['wmb'].wait()
            mb = jnp.dot(s8, wmod_v[:, 2 * D:6 * D], preferred_element_type=F32)
            mod_s[2] = mb[:, 0:D]
            mod_s[3] = mb[:, D:2 * D]
            mod_s[4] = 1.0 + mb[:, 2 * D:3 * D]
            gb = mb[:, 3 * D:4 * D]
            mod_s[5] = gb * (0.5 / GS)
            mod_s[6] = gb * jnp.broadcast_to(b2_v[...].astype(F32).reshape(1, D), (8, D))
            b1_s[...] = jnp.broadcast_to(b1_v[...].astype(F32).reshape(1, F), (8, F)) * GS

        def steady(waits):
            tn = jnp.minimum(i + 1, NT - 1)
            halo()
            qt = qkv_part(0) + qkv_part(1) + qkv_part(2)
            x1s, ys = [], []
            tk = pick(qt, len(lcs), L2START, L2STOP)
            for r0, t in zip(lcs, tk):
                if PACE_L2:
                    fence_a(t)
                x1b, y = l2(i - 1, r0, LC)
                x1s.append(x1b); ys.append(y)
            acc, mt = mlp_all(jnp.concatenate(ys, axis=0), waits)
            out(jnp.concatenate(x1s, axis=0), acc)
            nun = len(rcs) * (2 if SPLIT else 1)
            tk = pick(mt, nun, ASTART, ASTOP)
            u = 0
            for r0 in rcs:
                fence_qkv(tk[u]); u += 1
                p, rden = a_qk(r0, False)
                if SPLIT:
                    fence_qkv(tk[u]); u += 1
                a_pv(r0, p, rden)
            ot = wo_mm()
            tk = pick(ot, len(lcs), L1START, L1STOP)
            for r0, t in zip(lcs, tk):
                if PACE_L1:
                    fence_x(t)
                l1(tn, r0, LC)

        @pl.when(jnp.logical_and(i >= 1, i + 2 < NT))
        def _():
            xcopy(i + 2).start()

        @pl.when(jnp.logical_and(i >= 1, i + 1 < NT))
        def _():
            xcopy(i + 1).wait()

        if VAR1:
            @pl.when(i == 1)
            def _():
                steady(True)

            @pl.when(jnp.logical_and(i > 1, i < NT))
            def _():
                steady(None)
        else:
            @pl.when(jnp.logical_and(i > 0, i < NT))
            def _():
                steady(False)

        @pl.when(i == NT)
        def _():
            x1s, ys = [], []
            for r0 in lcs:
                x1b, y = l2(NT - 1, r0, LC)
                x1s.append(x1b); ys.append(y)
            acc, _ = mlp_all(jnp.concatenate(ys, axis=0), None)
            out(jnp.concatenate(x1s, axis=0), acc)

    def fn(A_x, A_wqkv, A_wo, B_x, B_w1, B_b1, B_w2, B_b2, c, w_mod):
        B, S, D = A_x.shape
        F = B_w1.shape[1]
        NT = S // TM
        NB = D // 128
        x = A_x.reshape(S, D)
        anyspec = pl.BlockSpec(memory_space=pl.ANY)
        out = pl.pallas_call(
            kernel,
            grid=(NT + 1,),
            in_specs=[anyspec] * 9,
            out_specs=pl.BlockSpec((TM, D), lambda i: (jnp.maximum(i - 1, 0), 0)),
            out_shape=jax.ShapeDtypeStruct((S, D), A_x.dtype),
            scratch_shapes=[
                pltpu.VMEM((S + 16, D), BF16),
                pltpu.VMEM((D, 3 * D), BF16),
                pltpu.VMEM((D, D), BF16),
                pltpu.VMEM((D, F), BF16),
                pltpu.VMEM((F,), BF16),
                pltpu.VMEM((F, D), BF16),
                pltpu.VMEM((D,), BF16),
                pltpu.VMEM((1, D), BF16),
                pltpu.VMEM((D, 6 * D), BF16),
                pltpu.VMEM((7, 8, D), F32),
                pltpu.VMEM((8, F), F32),
                pltpu.VMEM((D // 2, 3 * D), U32),
                pltpu.VMEM((NB, D, 128), F32),
                pltpu.VMEM((D // 2, D), U32),
                pltpu.VMEM((3 * NB, TM + HALO + 8, 128), F32),
                pltpu.VMEM((TM // 2, D), U32),
                pltpu.VMEM((TM + 8, D), F32),
                pltpu.VMEM((TM // 2, D), U32),
                pltpu.SMEM((1,), I32),
                pltpu.SemaphoreType.DMA((13 + NT,)),
            ],
            compiler_params=pltpu.CompilerParams(
                dimension_semantics=("arbitrary",),
                vmem_limit_bytes=100 * 1024 * 1024,
            ),
        )(x, A_wqkv, A_wo, B_w1, B_b1, B_w2, B_b2, c, w_mod)
        return out.reshape(B, S, D)
    return fn


pallas_adaLN_cond__sliding_local_dilated__mixer_channel_mlp__prompt_kernel = jax.jit(make_kernel(VAR1=1))
```

```python
import contextlib
import jax
import jax.numpy as jnp
from jax import lax
import jax.experimental.pallas as pl
import jax.experimental.pallas.tpu as pltpu

F32 = jnp.float32
BF16 = jnp.bfloat16
U32 = jnp.uint32
I32 = jnp.int32
H = 32
DH = 16
W = 8
DIL = 2
HALO = 16
EPS = 1e-5
LOG2E = 1.4426950408889634
GC0 = 0.7978845608028654
GC1 = GC0 * 0.044715
GS = GC1 ** (1.0 / 3.0)
GK = GC0 / GS


def _center(x):
    inv = 1.0 / x.shape[-1]
    m = jnp.sum(x, axis=-1, keepdims=True) * inv
    ms = jnp.sum(x * x, axis=-1, keepdims=True) * inv
    v = jnp.maximum(ms - m * m, 0.0)
    return x - m, lax.rsqrt(v + EPS)


def _spread(n, lo, hi):
    return [int(lo + (u * (hi - lo)) / n) for u in range(n)]


def make_kernel(TM=256, RC=16, FC=256, UN=2, ASTART=0.0, ASTOP=0.9, NTOK=4,
                LC=32, L2START=0.0, L2STOP=0.5, L1START=0.5, L1STOP=0.9, WSPLITS=(0, 1, 3, 6),
                SEGMARGIN=5, A0STOP=0.7, L20STOP=0.6, ESPLIT=(64, 192), EFCS=(1792,), MERGE0=1,
                SCOPES=0, ONLY=None,
                DMAORD=('x0', 'c', 'wma', 'wq', 'wk', 'wv', 'x1', 'wo', 'b1', 'b2', 'wmb', 'W', 'wmc', 'x2')):
    ns = jax.named_scope if SCOPES else (lambda name: contextlib.nullcontext())

    def kernel(x_hbm, wqkv_hbm, wo_hbm, w1_hbm, b1_hbm, w2_hbm, b2_hbm, c_hbm, wmod_hbm,
               out_hbm,
               x_s, wqkv_v, wo_v, w1_v, b1_v, w2_v, b2_v, c_v, wmod_v,
               mod_s, b1_s, s8_s, wqkv_p, wo_f, wo_p, qkv_s, qkv0_s, a_s, y_s, z_s, sem, osem, *ho_b):
        h_b, o_b = ho_b[:UN + 1], ho_b[UN + 1:]
        i = pl.program_id(0)
        S, D = x_hbm.shape
        NT = S // TM
        NBLK = (NT - 2) // UN
        F = w1_hbm.shape[-1]
        NB = D // 128
        QO, KO, VO = 0, NB, 2 * NB
        fcs = [(f0, FC) for f0 in range(0, F, FC)]
        wb = [fcs[k][0] for k in WSPLITS] + [F]

        srcdst = {}
        def defcopy(name, src, dst):
            srcdst[name] = (src, dst, len(srcdst))
        defcopy('c', c_hbm, c_v)
        defcopy('b1', b1_hbm, b1_v)
        defcopy('b2', b2_hbm, b2_v)
        for p, n in enumerate(('wq', 'wk', 'wv')):
            defcopy(n, wqkv_hbm.at[:, p * D:(p + 1) * D], wqkv_v.at[:, p * D:(p + 1) * D])
        defcopy('wma', wmod_hbm.at[:, 0:2 * D], wmod_v.at[:, 0:2 * D])
        defcopy('wmb', wmod_hbm.at[:, 2 * D:5 * D], wmod_v.at[:, 2 * D:5 * D])
        defcopy('wmc', wmod_hbm.at[:, 5 * D:6 * D], wmod_v.at[:, 5 * D:6 * D])
        defcopy('wo', wo_hbm, wo_v)
        for k in range(len(WSPLITS)):
            defcopy(f'w1{k}', w1_hbm.at[:, wb[k]:wb[k + 1]], w1_v.at[:, wb[k]:wb[k + 1]])
            defcopy(f'w2{k}', w2_hbm.at[wb[k]:wb[k + 1], :], w2_v.at[wb[k]:wb[k + 1], :])
        for t in range(3):
            defcopy(f'x{t}', x_hbm.at[t * TM:(t + 1) * TM, :], x_s.at[t * TM:(t + 1) * TM, :])
        defcopy('xr', x_hbm.at[3 * TM:S, :], x_s.at[3 * TM:S, :])

        def cp(name):
            src, dst, k = srcdst[name]
            return pltpu.make_async_copy(src, dst, sem.at[k])

        def wait(*names):
            with ns('w_' + names[0]):
                for n in names:
                    cp(n).wait()

        def rows(t, r0, n, mult=16):
            if isinstance(t, int):
                return pl.ds(t * TM + r0, n)
            return pl.ds(pl.multiple_of(t * TM + r0, mult), n)

        def ocopy(t, r0, n, k):
            return pltpu.make_async_copy(y_s.at[rows(t, r0, n), :], out_hbm.at[rows(t, r0, n), :], osem.at[k])

        def modv(k, n):
            return jnp.broadcast_to(mod_s[k, 0:1, :], (n, D))

        def zero():
            return z_s[0]

        def fence_a(tok):
            row = pl.multiple_of(TM + 8 * zero(), 8)
            a_s[pl.ds(row, 8), 0:128] = tok

        def fence_x(tok):
            row = pl.multiple_of(S + 16 * zero(), 16)
            x_s[pl.ds(row, 16), 0:128] = jnp.concatenate([tok, tok], axis=0).astype(BF16)

        def tokzero(tok):
            return pltpu.bitcast(tok, I32) & jnp.full((8, 128), zero(), I32)

        def tie(v, tz):
            t = jnp.concatenate([tz] * (v.shape[0] // 8), axis=0) if v.shape[0] > 8 else tz
            return pltpu.bitcast(pltpu.bitcast(v, I32) | t, v.dtype)

        def perm_cols(p):
            lane = lax.broadcasted_iota(I32, (D // 2, 128), 1)
            b = (lane >> 2) & 3
            blk = [pltpu.bitcast(wqkv_v[:, p * D + k * 128:p * D + (k + 1) * 128], U32) for k in range(NB)]
            prev = None
            for j in range(NB):
                m = jnp.where(b == 0, blk[j], blk[(j + 1) % NB])
                m = jnp.where(b == 2, blk[(j + 2) % NB], m)
                m = jnp.where(b == 3, blk[(j + 3) % NB], m)
                if prev is not None:
                    m = tie(m, tokzero(prev))
                idx = (((lane >> 1) & 7) * 16 + ((((lane >> 4) & 3) + (NB - j)) & 3) * 4
                       + (lane >> 6) * 2 + (lane & 1))
                r = jnp.take_along_axis(m, idx, axis=1)
                wqkv_p[:, p * D + j * 128:p * D + (j + 1) * 128] = r
                prev = r[D // 2 - 8:D // 2, :]

        def perm_wo():
            for k in range(NB):
                wo_f[k] = pltpu.bitcast(wo_v[:, k * 128:(k + 1) * 128], U32)
            for j in range(NB):
                for e1 in range(2):
                    for ii in range(4):
                        g = (ii - j) % 4
                        r = j * 64 + e1 * 32 + ii * 8
                        for k in range(NB):
                            wo_p[r:r + 8, k * 128:(k + 1) * 128] = wo_f[k, pl.ds(ii * 64 + g * 2 + e1, 8, stride=8), :]

        def xrows(t, r0, n):
            return x_s[rows(t, r0, n), :].astype(F32)

        def l1_mod(hbuf, xn, r0, n):
            h = xn * modv(1, n) + modv(0, n)
            hbuf[r0 // 2:(r0 + n) // 2, :] = pltpu.bitcast(h.astype(BF16), U32)

        def l1(hbuf, t, r0, n):
            xc, rs = _center(xrows(t, r0, n))
            l1_mod(hbuf, xc * rs, r0, n)

        def toks_of(r, cstep):
            n = r.shape[0]
            return [r[k:k + 8, c:c + 128] for c in range(0, r.shape[1], cstep) for k in range(0, n, n // NTOK)]

        def qkv_part(hbuf, buf, p):
            h = pltpu.bitcast(hbuf[...], BF16)
            r = jnp.dot(h, pltpu.bitcast(wqkv_p[:, p * D:(p + 1) * D], BF16), preferred_element_type=F32)
            if p == 0:
                r = r * ((DH ** -0.5) * LOG2E)
            for j in range(NB):
                buf[p * NB + j, HALO:HALO + TM, :] = r[:, j * 128:(j + 1) * 128]
            return toks_of(r, 128)

        def attn(buf, o_s, r0, first, tok=None):
            q = [buf[QO + j, HALO + r0:HALO + r0 + RC, :] for j in range(NB)]
            if tok is not None:
                tz = tokzero(tok)
                q = [tie(v, tz) for v in q]
            swap = lax.broadcasted_iota(I32, (RC, 128), 1) ^ 1
            lg = []
            for w in range(W):
                st = HALO + r0 - DIL * w
                acc = q[0] * buf[KO, st:st + RC, :]
                for j in range(1, NB):
                    acc = acc + q[j] * buf[KO + j, st:st + RC, :]
                acc = acc + pltpu.roll(acc, 64, 1)
                acc = acc + jnp.take_along_axis(acc, swap, axis=1)
                if first and r0 < HALO and w > 0:
                    row = r0 + lax.broadcasted_iota(I32, (RC, 128), 0)
                    acc = jnp.where(row >= DIL * w, acc, -1e9 * LOG2E)
                lg.append(acc)
            m = lg[0]
            for w in range(1, W):
                m = jnp.maximum(m, lg[w])
            p = [jnp.exp2(l - m) for l in lg]
            den = p[0]
            for w in range(1, W):
                den = den + p[w]
            rden = pl.reciprocal(den, approx=True)
            for j in range(NB):
                st = HALO + r0
                acc = p[0] * buf[VO + j, st:st + RC, :]
                for w in range(1, W):
                    st = HALO + r0 - DIL * w
                    acc = acc + p[w] * buf[VO + j, st:st + RC, :]
                o_s[r0 // 2:(r0 + RC) // 2, j * 128:(j + 1) * 128] = pltpu.bitcast((acc * rden).astype(BF16), U32)

        rcs = list(range(0, TM, RC))
        lcs = list(range(0, TM, LC))
        nun = len(rcs)

        def wo_mm(o_s):
            a = jnp.dot(pltpu.bitcast(o_s[...], BF16), pltpu.bitcast(wo_p[...], BF16), preferred_element_type=F32)
            a_s[0:TM, :] = a

        def l2(t, r0, n):
            x1 = xrows(t, r0, n) + modv(2, n) * a_s[r0:r0 + n, :]
            xc, rs = _center(x1)
            h2 = (xc * rs) * modv(4, n) + modv(3, n)
            hc, rs2 = _center(h2)
            y = (hc * (rs2 * GS)).astype(BF16)
            return x1, y

        def mlp(y, f0, fc):
            n = y.shape[0]
            z = jnp.dot(y, w1_v[:, f0:f0 + fc], preferred_element_type=F32)
            z = z + jnp.broadcast_to(b1_s[0:1, f0:f0 + fc], (n, fc))
            g = (z + z * jnp.tanh(z * (z * z + GK))).astype(BF16)
            part = jnp.dot(g, w2_v[f0:f0 + fc, :], preferred_element_type=F32)
            return part, toks_of(z, 128) + toks_of(part, max(128, min(D, 65536 // fc)))

        def out(t, x1, acc, r0, n):
            y_s[rows(t, r0, n), :] = (x1 + (modv(5, n) * acc + modv(6, n))).astype(BF16)

        def mod_mm(c0, c1):
            return jnp.dot(s8_s[0:8, :].astype(BF16), wmod_v[:, c0:c1], preferred_element_type=F32)

        @pl.when(i == 0)
        def _():
          if ONLY not in (None, 'p'):
              return
          with ns('prologue'):
            h0 = h_b[UN - 1]
            z_s[0] = 0
            for n in DMAORD:
                if n == 'W':
                    for k in range(len(WSPLITS)):
                        cp(f'w1{k}').start()
                        cp(f'w2{k}').start()
                else:
                    cp(n).start()
            cp('xr').start()
            qkv0_s[KO:, 0:HALO, :] = jnp.zeros((2 * NB, HALO, 128), F32)
            wait('x0', 'c')
            c = c_v[...].astype(F32)
            s8_s[...] = jnp.broadcast_to(c * jax.nn.sigmoid(c), (8, D))
            for r0 in lcs:
                xc, rs = _center(xrows(0, r0, LC))
                a_s[r0:r0 + LC, :] = xc * rs
            wait('wma')
            ma = mod_mm(0, 2 * D)
            mod_s[0] = ma[:, 0:D]
            mod_s[1] = 1.0 + ma[:, D:2 * D]
            for r0 in lcs:
                l1_mod(h0, a_s[r0:r0 + LC, :], r0, LC)
            wait('wq')
            perm_cols(0)
            qkv_part(h0, qkv0_s, 0)
            wait('wk')
            perm_cols(1)
            qkv_part(h0, qkv0_s, 1)
            wait('wv', 'x1')
            perm_cols(2)
            qkv_part(h0, qkv0_s, 2)
            for r0 in lcs:
                l1(h_b[UN], 1, r0, LC)

        def tile(t, hcur, hnext, tnext, o_s, first):
            x1s, ys = [], []
            if first:
                wait('wo')
                perm_wo()
                qkv_s[KO:, 0:HALO, :] = qkv0_s[KO:, TM:TM + HALO, :]
                qt = qkv_part(hcur, qkv_s, 0) + qkv_part(hcur, qkv_s, 1)
                for u, k in enumerate(_spread(nun, 0, A0STOP * len(qt))):
                    attn(qkv0_s, o_b[1], rcs[u], True, qt[k] if u > 0 else None)
                wo_mm(o_b[1])
                wait('wmb', 'b1')
                if MERGE0:
                    wait('w10', 'w20')
                mb = mod_mm(2 * D, 5 * D)
                mod_s[2] = mb[:, 0:D]
                mod_s[3] = mb[:, D:2 * D]
                mod_s[4] = 1.0 + mb[:, 2 * D:3 * D]
                b1_s[...] = jnp.broadcast_to(b1_v[...].astype(F32).reshape(1, F), (8, F)) * GS
                qt = qkv_part(hcur, qkv_s, 2)
                l2i = _spread(len(lcs), 0, L20STOP * len(qt))
            else:
                qkv_s[KO:, 0:HALO, :] = qkv_s[KO:, TM:TM + HALO, :]
                qt = qkv_part(hcur, qkv_s, 0) + qkv_part(hcur, qkv_s, 1) + qkv_part(hcur, qkv_s, 2)
                l2i = _spread(len(lcs), L2START * len(qt), L2STOP * len(qt))
            for r0, k in zip(lcs, l2i):
                fence_a(qt[k])
                x1, y = l2(t - 1, r0, LC)
                x1s.append(x1); ys.append(y)
            if not first:
                for r0, k in zip(lcs, _spread(len(lcs), L1START * len(qt), L1STOP * len(qt))):
                    fence_x(qt[k])
                    l1(hnext, tnext, r0, LC)
            y = jnp.concatenate(ys, axis=0)
            tpc = NTOK * (FC // 128 + max(1, FC * D // 65536))
            ntok = tpc * len(fcs)
            lidx = []
            if first:
                ends = [k * tpc for k in WSPLITS[1:]]
                usable = [u for u in range(int(ASTOP * ntok)) if not any(0 < e - u <= SEGMARGIN for e in ends)]
                aidx = [usable[k] for k in _spread(nun, 0, len(usable))]
                lidx = _spread(len(lcs), WSPLITS[-1] * tpc, ntok)
            else:
                aidx = _spread(nun, ASTART * ntok, ASTOP * ntok)
            acc = None
            ua = 0
            ul = 0
            for n, (f0, fc) in enumerate(fcs):
                if first and n in WSPLITS:
                    k = WSPLITS.index(n)
                    if not (MERGE0 and k == 0):
                        wait(f'w1{k}', f'w2{k}')
                    if n == WSPLITS[-1]:
                        wait('wmc', 'b2', 'x2')
                        gb = mod_mm(5 * D, 6 * D)
                        mod_s[5] = gb * (0.5 / GS)
                        mod_s[6] = gb * jnp.broadcast_to(b2_v[...].astype(F32).reshape(1, D), (8, D))
                part, tk = mlp(y, f0, fc)
                assert len(tk) == tpc
                acc = part if acc is None else acc + part
                while ua < nun and aidx[ua] // tpc == n:
                    attn(qkv_s, o_s, rcs[ua], False, tk[aidx[ua] % tpc])
                    ua += 1
                while ul < len(lidx) and lidx[ul] // tpc == n:
                    fence_x(tk[lidx[ul] % tpc])
                    l1(hnext, tnext, lcs[ul], LC)
                    ul += 1
            assert ua == nun
            out(t - 1, jnp.concatenate(x1s, axis=0), acc, 0, TM)
            wo_mm(o_s)

        @pl.when(i == 1)
        def _():
            if ONLY in (None, 's1'):
              with ns('step1'):
                tile(1, h_b[UN], h_b[0], 2, o_b[0], True)
                ocopy(0, 0, TM, 0).start()

        @pl.when(i == 2)
        def _():
            cp('xr').wait()

        @pl.when(jnp.logical_and(i > 1, i < NBLK + 2))
        def _():
            if ONLY in (None, 's'):
              with ns('steady'):
                t0 = 2 + (i - 2) * UN
                for u in range(UN):
                    tn = t0 + u + 1
                    if u == UN - 1:
                        tn = jnp.minimum(tn, NT - 1)
                    tile(t0 + u, h_b[u], h_b[(u + 1) % UN], tn, o_b[u], False)
                ocopy(t0 - 1, 0, UN * TM, i - 1).start()

        @pl.when(i == NBLK + 2)
        def _():
          if ONLY not in (None, 'e'):
              return
          with ns('epilogue'):
            h0 = 0
            prev = None
            for e, hm in enumerate(ESPLIT):
                x1s, ys = [], []
                for r0 in range(h0, h0 + hm, LC):
                    if prev is not None:
                        fence_a(prev)
                    x1, y = l2(NT - 1, r0, LC)
                    prev = None
                    x1s.append(x1); ys.append(y)
                y = jnp.concatenate(ys, axis=0)
                acc = None
                efcs = fcs
                if hm < 128:
                    efcs = [(sum(EFCS[:k]), EFCS[k]) for k in range(len(EFCS))]
                for n, (f0, fc) in enumerate(efcs):
                    part, tk = mlp(y, f0, fc)
                    if n == 0 and e == 0:
                        prev = tk[0]
                    acc = part if acc is None else acc + part
                out(NT - 1, jnp.concatenate(x1s, axis=0), acc, h0, hm)
                h0 += hm
            ocopy(NT - 1, 0, TM, NBLK + 1).start()
            ocopy(0, 0, TM, 0).wait()
            for k in range(NBLK):
                ocopy(1 + k * UN, 0, UN * TM, k + 1).wait()
            ocopy(NT - 1, 0, TM, NBLK + 1).wait()

    def fn(A_x, A_wqkv, A_wo, B_x, B_w1, B_b1, B_w2, B_b2, c, w_mod):
        B, S, D = A_x.shape
        F = B_w1.shape[1]
        NT = S // TM
        assert (NT - 2) % UN == 0
        NBLK = (NT - 2) // UN
        NB = D // 128
        x = A_x.reshape(S, D)
        anyspec = pl.BlockSpec(memory_space=pl.ANY)
        out = pl.pallas_call(
            kernel,
            grid=(NBLK + 3,),
            in_specs=[anyspec] * 9,
            out_specs=anyspec,
            out_shape=jax.ShapeDtypeStruct((S, D), A_x.dtype),
            scratch_shapes=[
                pltpu.VMEM((S + 16, D), BF16),
                pltpu.VMEM((D, 3 * D), BF16),
                pltpu.VMEM((D, D), BF16),
                pltpu.VMEM((D, F), BF16),
                pltpu.VMEM((F,), BF16),
                pltpu.VMEM((F, D), BF16),
                pltpu.VMEM((D,), BF16),
                pltpu.VMEM((1, D), BF16),
                pltpu.VMEM((D, 6 * D), BF16),
                pltpu.VMEM((7, 8, D), F32),
                pltpu.VMEM((8, F), F32),
                pltpu.VMEM((8, D), F32),
                pltpu.VMEM((D // 2, 3 * D), U32),
                pltpu.VMEM((NB, D // 2, 128), U32),
                pltpu.VMEM((D // 2, D), U32),
                pltpu.VMEM((3 * NB, TM + HALO, 128), F32),
                pltpu.VMEM((3 * NB, TM + HALO, 128), F32),
                pltpu.VMEM((TM + 8, D), F32),
                pltpu.VMEM((S, D), BF16),
                pltpu.SMEM((1,), I32),
                pltpu.SemaphoreType.DMA((14 + 2 * len(WSPLITS),)),
                pltpu.SemaphoreType.DMA((NBLK + 2,)),
            ] + [pltpu.VMEM((TM // 2, D), U32)] * (UN + 1 + max(UN, 2)),
            compiler_params=pltpu.CompilerParams(
                dimension_semantics=("arbitrary",),
                vmem_limit_bytes=100 * 1024 * 1024,
            ),
        )(x, A_wqkv, A_wo, B_w1, B_b1, B_w2, B_b2, c, w_mod)
        return out.reshape(B, S, D)
    return fn


pallas_adaLN_cond__sliding_local_dilated__mixer_channel_mlp__prompt_kernel = jax.jit(make_kernel(LC=16, L1STOP=1.0, NTOK=8, ASTOP=0.8, ASTART=0.03, L2STOP=0.45, SEGMARGIN=10))
```

```python
import contextlib
import jax
import jax.numpy as jnp
from jax import lax
import jax.experimental.pallas as pl
import jax.experimental.pallas.tpu as pltpu

F32 = jnp.float32
BF16 = jnp.bfloat16
U32 = jnp.uint32
I32 = jnp.int32
H = 32
DH = 16
W = 8
DIL = 2
HALO = 16
EPS = 1e-5
LOG2E = 1.4426950408889634
GC0 = 0.7978845608028654
GC1 = GC0 * 0.044715
GS = GC1 ** (1.0 / 3.0)
GK = GC0 / GS


def _center(x):
    inv = 1.0 / x.shape[-1]
    m = jnp.sum(x, axis=-1, keepdims=True) * inv
    ms = jnp.sum(x * x, axis=-1, keepdims=True) * inv
    v = jnp.maximum(ms - m * m, 0.0)
    return x - m, lax.rsqrt(v + EPS)


def _spread(n, lo, hi):
    return [int(lo + (u * (hi - lo)) / n) for u in range(n)]


def make_kernel(TM=256, RC=16, FC=256, UN=2, ASTART=0.03, ASTOP=0.8, NTOK=8,
                LC=16, L2START=0.0, L2STOP=0.45, L1START=0.5, L1STOP=1.0, WSPLITS=(0, 1, 3, 5),
                SEGMARGIN=10, A0START=0.0, A0STOP=0.3, A0FREE=4, MERGE0=1, A0LAG=2, L2LAG=2, PACKW=1, SFCS=(512, 512, 512, 256), CHAIN=2, L1CHAIN=2, L1PER=4, EDMA=1, L10STOP=0.75, L10FREE=4, QCUT=3, XB=0, QV=1, L20FREE=0, NEWTON=0, CHAIN1=2, A1START=0.02, L12M=16, L20STOP=0.3, A1STOP=0.55, OLAST=0,
                RH=64, LHSTART=0.1, LHSTOP=0.3, ESPLIT=(160, 32), EFCS=(1792,), EL2STOP=0.3,
                SCOPES=0, ONLY=None,
                DMAORD=('x0', 'c', 'wma', 'wq', 'wk', 'wv', 'x1', 'wo', 'b1', 'b2', 'wmb', 'W', 'wmc', 'x2')):
    ns = jax.named_scope if SCOPES else (lambda name: contextlib.nullcontext())

    def kernel(x_hbm, wqkv_hbm, wo_hbm, w1_hbm, b1_hbm, w2_hbm, b2_hbm, c_hbm, wmod_hbm,
               out_hbm,
               x_s, wqkv_v, wo_v, w1_v, b1_v, w2_v, b2_v, c_v, wmod_v,
               mod_s, b1_s, s8_s, wqkv_p, wo_f, wo_p, qkv_s, qkv0_s, a_s, y_s, w1_p, w2_p, z_s, sem, osem, *bufs):
        h_b = bufs[:UN + 1]
        o_b = bufs[UN + 1:2 * UN + 2]
        yh_b = bufs[2 * UN + 2:3 * UN + 2]
        xh_b = bufs[3 * UN + 2:4 * UN + 2]
        i = pl.program_id(0)
        S, D = x_hbm.shape
        NT = S // TM
        NBLK = (NT - 2) // UN
        F = w1_hbm.shape[-1]
        NB = D // 128
        QO, KO, VO = 0, NB, 2 * NB
        fcs = [(f0, FC) for f0 in range(0, F, FC)]
        wb = [fcs[k][0] for k in WSPLITS] + [F]
        sfcs = [(sum(SFCS[:k]), SFCS[k]) for k in range(len(SFCS))]

        srcdst = {}
        def defcopy(name, src, dst):
            srcdst[name] = (src, dst, len(srcdst))
        defcopy('c', c_hbm, c_v)
        defcopy('b1', b1_hbm, b1_v)
        defcopy('b2', b2_hbm, b2_v)
        for p, n in enumerate(('wq', 'wk', 'wv')):
            defcopy(n, wqkv_hbm.at[:, p * D:(p + 1) * D], wqkv_v.at[:, p * D:(p + 1) * D])
        defcopy('wma', wmod_hbm.at[:, 0:2 * D], wmod_v.at[:, 0:2 * D])
        defcopy('wmb', wmod_hbm.at[:, 2 * D:5 * D], wmod_v.at[:, 2 * D:5 * D])
        defcopy('wmc', wmod_hbm.at[:, 5 * D:6 * D], wmod_v.at[:, 5 * D:6 * D])
        defcopy('wo', wo_hbm, wo_v)
        for k in range(len(WSPLITS)):
            defcopy(f'w1{k}', w1_hbm.at[:, wb[k]:wb[k + 1]], w1_v.at[:, wb[k]:wb[k + 1]])
            defcopy(f'w2{k}', w2_hbm.at[wb[k]:wb[k + 1], :], w2_v.at[wb[k]:wb[k + 1], :])
        for t in range(3):
            defcopy(f'x{t}', x_hbm.at[t * TM:(t + 1) * TM, :], x_s.at[t * TM:(t + 1) * TM, :])
        defcopy('xr', x_hbm.at[3 * TM:S, :], x_s.at[3 * TM:S, :])

        def cp(name):
            src, dst, k = srcdst[name]
            return pltpu.make_async_copy(src, dst, sem.at[k])

        def wait(*names):
            with ns('w_' + names[0]):
                for n in names:
                    cp(n).wait()

        def rows(t, r0, n, mult=16):
            if isinstance(t, int):
                return pl.ds(t * TM + r0, n)
            return pl.ds(pl.multiple_of(t * TM + r0, mult), n)

        def ocopy(t, r0, n, k):
            return pltpu.make_async_copy(y_s.at[rows(t, r0, n), :], out_hbm.at[rows(t, r0, n), :], osem.at[k])

        def rep8(v, n):
            return v if n == 8 else jnp.concatenate([v] * (n // 8), axis=0)

        def modv(k, n):
            return rep8(mod_s[k], n)

        def zero():
            return z_s[0]

        def fence_a(tok):
            row = pl.multiple_of(TM + 8 * zero(), 8)
            a_s[pl.ds(row, 8), 0:128] = tok

        def fence_x(tok):
            row = pl.multiple_of(S + 16 * zero(), 16)
            x_s[pl.ds(row, 16), 0:128] = jnp.concatenate([tok, tok], axis=0).astype(BF16)

        def tokzero(tok):
            return pltpu.bitcast(tok, I32) & jnp.full((8, 128), zero(), I32)

        def tie(v, tz):
            t = jnp.concatenate([tz] * (v.shape[0] // 8), axis=0) if v.shape[0] > 8 else tz
            if v.shape[1] > 128:
                t = jnp.concatenate([t] * (v.shape[1] // 128), axis=1)
            return pltpu.bitcast(pltpu.bitcast(v, I32) | t, v.dtype)

        def perm_cols(p):
            lane = lax.broadcasted_iota(I32, (D // 2, 128), 1)
            b = (lane >> 2) & 3
            blk = [pltpu.bitcast(wqkv_v[:, p * D + k * 128:p * D + (k + 1) * 128], U32) for k in range(NB)]
            prev = None
            for j in range(NB):
                m = jnp.where(b == 0, blk[j], blk[(j + 1) % NB])
                m = jnp.where(b == 2, blk[(j + 2) % NB], m)
                m = jnp.where(b == 3, blk[(j + 3) % NB], m)
                if prev is not None:
                    m = tie(m, tokzero(prev))
                idx = (((lane >> 1) & 7) * 16 + ((((lane >> 4) & 3) + (NB - j)) & 3) * 4
                       + (lane >> 6) * 2 + (lane & 1))
                r = jnp.take_along_axis(m, idx, axis=1)
                wqkv_p[:, p * D + j * 128:p * D + (j + 1) * 128] = r
                prev = r[D // 2 - 8:D // 2, :]

        def perm_wo():
            for k in range(NB):
                wo_f[k] = pltpu.bitcast(wo_v[:, k * 128:(k + 1) * 128], U32)
            for k in range(NB):
                for j in range(NB):
                    for e1 in range(2):
                        for ii in range(4):
                            g = (ii - j) % 4
                            r = j * 64 + e1 * 32 + ii * 8
                            wo_p[r:r + 8, k * 128:(k + 1) * 128] = wo_f[k, pl.ds(ii * 64 + g * 2 + e1, 8, stride=8), :]

        def xrows(t, r0, n):
            return x_s[rows(t, r0, n), :].astype(F32)

        def l1_mod(hbuf, xn, r0, n):
            h = xn * modv(1, n) + modv(0, n)
            hv = pltpu.bitcast(h.astype(BF16), U32)
            hbuf[r0 // 2:(r0 + n) // 2, :] = hv
            return hv[0:8, D - 128:D]

        def l1(hbuf, t, r0, n):
            xc, rs = _center(xrows(t, r0, n))
            return l1_mod(hbuf, xc * rs, r0, n)

        def toks_of(r, cstep):
            n = r.shape[0]
            step = max(8, (TM // NTOK))
            return [r[k:k + 8, c:c + 128] for c in range(0, r.shape[1], cstep) for k in range(0, n, step)]

        def qkv_cols(hbuf, buf, j0, j1):
            h = pltpu.bitcast(hbuf[...], BF16)
            r = jnp.dot(h, pltpu.bitcast(wqkv_p[:, j0 * 128:j1 * 128], BF16), preferred_element_type=F32)
            if j0 < NB:
                assert j1 <= NB
                r = r * ((DH ** -0.5) * LOG2E)
            for j in range(j0, j1):
                buf[j, HALO:HALO + TM, :] = r[:, (j - j0) * 128:(j - j0 + 1) * 128]
            return toks_of(r, 128)

        def qkv_part(hbuf, buf, p):
            return qkv_cols(hbuf, buf, p * NB, (p + 1) * NB)

        def qkv_range(hbuf, buf, j0, j1):
            tk = []
            if j0 < NB:
                tk += qkv_cols(hbuf, buf, j0, min(j1, NB))
                j0 = NB
            if j1 > j0:
                tk += qkv_cols(hbuf, buf, j0, j1)
            return tk

        def attn1(buf, r0, tok=None, dep=None):
            q = [buf[QO + j, HALO + r0:HALO + r0 + RC, :] for j in range(NB)]
            if tok is not None:
                tz = tokzero(tok)
                if dep is not None:
                    tz = tz | tokzero(dep)
                q = [tie(v, tz) for v in q]
            lg = []
            for w in range(W):
                st = HALO + r0 - DIL * w
                acc = q[0] * buf[KO, st:st + RC, :]
                for j in range(1, NB):
                    acc = acc + q[j] * buf[KO + j, st:st + RC, :]
                lg.append(acc)
            rl = [pltpu.roll(a, 64, 1) for a in lg]
            return [a + b for a, b in zip(lg, rl)]

        def attn2(buf, o_s, r0, first, lg):
            swap = lax.broadcasted_iota(I32, (RC, 128), 1) ^ 1
            sw = [jnp.take_along_axis(a, swap, axis=1) for a in lg]
            lg = [a + b for a, b in zip(lg, sw)]
            if first and r0 < HALO:
                row = r0 + lax.broadcasted_iota(I32, (RC, 128), 0)
                lg = [lg[0]] + [jnp.where(row >= DIL * w, lg[w], -1e9 * LOG2E) for w in range(1, W)]
            m = lg[0]
            for w in range(1, W):
                m = jnp.maximum(m, lg[w])
            p = [jnp.exp2(l - m) for l in lg]
            den = p[0]
            for w in range(1, W):
                den = den + p[w]
            rden = pl.reciprocal(den, approx=True)
            if NEWTON:
                rden = rden * (2.0 - den * rden)
            for j in range(NB):
                st = HALO + r0
                acc = p[0] * buf[VO + j, st:st + RC, :]
                for w in range(1, W):
                    st = HALO + r0 - DIL * w
                    acc = acc + p[w] * buf[VO + j, st:st + RC, :]
                ov = pltpu.bitcast((acc * rden).astype(BF16), U32)
                o_s[r0 // 2:(r0 + RC) // 2, j * 128:(j + 1) * 128] = ov
            return ov

        def attn(buf, o_s, r0, first, tok=None, dep=None):
            return attn2(buf, o_s, r0, first, attn1(buf, r0, tok, dep))

        def pipelined(n, lag, stage1, stage2):
            mid = {}
            res = []
            for u in range(n + lag):
                if u < n:
                    mid[u] = stage1(u)
                if u >= lag:
                    res.append(stage2(u - lag, mid.pop(u - lag)))
            return res

        rcs = list(range(0, TM, RC))
        lcs = list(range(0, TM, LC))
        nun = len(rcs)

        def l2_a(x1, n):
            xc, rs = _center(x1)
            return x1, (xc * rs) * modv(4, n) + modv(3, n)

        def l2_b(h2):
            hc, rs2 = _center(h2)
            return (hc * (rs2 * GS)).astype(BF16)

        def l2_units(t, cs, toks):
            def s1(k):
                if toks[k] is not None:
                    fence_a(toks[k])
                r0 = cs[k]
                return l2_a(xrows(t, r0, LC) + modv(2, LC) * a_s[r0:r0 + LC, :], LC)
            res = pipelined(len(cs), L2LAG, s1, lambda k, m: (m[0], l2_b(m[1])))
            return [r[0] for r in res], [r[1] for r in res]

        def wo_mm(o_s, t=None, u=None):
            wo = pltpu.bitcast(wo_p[...], BF16)
            if t is None or RH == 0:
                a_s[0:TM, :] = jnp.dot(pltpu.bitcast(o_s[...], BF16), wo, preferred_element_type=F32)
                return
            ah = jnp.dot(pltpu.bitcast(o_s[0:RH // 2, :], BF16), wo, preferred_element_type=F32)
            a = jnp.dot(pltpu.bitcast(o_s[RH // 2:TM // 2, :], BF16), wo, preferred_element_type=F32)
            a_s[RH:TM, :] = a
            tk = toks_of(a, 128)
            hcs = list(range(0, RH, LC))
            ks = _spread(len(hcs), LHSTART * len(tk), LHSTOP * len(tk))
            def s1(k):
                r0 = hcs[k]
                x1 = xrows(t, r0, LC) + modv(2, LC) * tie(ah[r0:r0 + LC, :], tokzero(tk[ks[k]]))
                xh_b[u][r0:r0 + LC, :] = x1
                return l2_a(x1, LC)[1]
            def s2(k, h2):
                r0 = hcs[k]
                yh_b[u][r0 // 2:(r0 + LC) // 2, :] = pltpu.bitcast(l2_b(h2), U32)
            pipelined(len(hcs), L2LAG, s1, s2)

        def mlp(y, f0, fc, raw=False):
            n = y.shape[0]
            if raw or not PACKW:
                w1c = w1_v[:, f0:f0 + fc]
                w2c = w2_v[f0:f0 + fc, :]
                if PACKW:
                    w1_p[:, f0:f0 + fc] = pltpu.bitcast(w1c, U32)
                    w2_p[f0 // 2:(f0 + fc) // 2, :] = pltpu.bitcast(w2c, U32)
            else:
                w1c = pltpu.bitcast(w1_p[:, f0:f0 + fc], BF16)
                w2c = pltpu.bitcast(w2_p[f0 // 2:(f0 + fc) // 2, :], BF16)
            z = jnp.dot(y, w1c, preferred_element_type=F32)
            z = z + rep8(b1_s[:, f0:f0 + fc], n)
            g = (z + z * jnp.tanh(z * (z * z + GK))).astype(BF16)
            part = jnp.dot(g, w2c, preferred_element_type=F32)
            return part, toks_of(z, 128) + toks_of(part, max(128, min(D, 65536 // fc)))

        def out(t, x1, acc, r0, n):
            y_s[rows(t, r0, n), :] = (x1 + (modv(5, n) * acc + modv(6, n))).astype(BF16)

        def mod_mm(c0, c1):
            return jnp.dot(s8_s[0:8, :].astype(BF16), wmod_v[:, c0:c1], preferred_element_type=F32)

        tpc = NTOK * (FC // 128 + max(1, FC * D // 65536))
        ntok = tpc * len(fcs)

        @pl.when(i == 0)
        def _():
            z_s[0] = 0
            for n in DMAORD:
                if n == 'W':
                    for k in range(len(WSPLITS)):
                        cp(f'w1{k}').start()
                        cp(f'w2{k}').start()
                else:
                    cp(n).start()
            cp('xr').start()
            qkv0_s[KO:, 0:HALO, :] = jnp.zeros((2 * NB, HALO, 128), F32)

        @pl.when(i == 1)
        def _():
          if ONLY not in (None, 'p'):
              return
          with ns('startup'):
            h0, h1 = h_b[UN - 1], h_b[UN]
            wait('x0', 'c')
            c = c_v[...].astype(F32)
            s8_s[...] = jnp.broadcast_to(c * jax.nn.sigmoid(c), (8, D))
            for r0 in lcs:
                xc, rs = _center(xrows(0, r0, LC))
                a_s[r0:r0 + LC, :] = xc * rs
            wait('wma')
            ma = mod_mm(0, 2 * D)
            mod_s[0] = ma[:, 0:D]
            mod_s[1] = 1.0 + ma[:, D:2 * D]
            for r0 in lcs:
                l1_mod(h0, a_s[r0:r0 + LC, :], r0, LC)
            wait('wq')
            perm_cols(0)
            qkv_range(h0, qkv0_s, 0, QCUT)
            wait('wk')
            perm_cols(1)
            qkv_range(h0, qkv0_s, QCUT, NB + QCUT)
            if XB == 0:
                wait('wv', 'x1')
                perm_cols(2)
                qt = qkv_range(h0, qkv0_s, NB + QCUT, 3 * NB)
            else:
                wait('wv')
                perm_cols(2)
                qkv_range(h0, qkv0_s, NB + QCUT, 2 * NB + XB)
                wait('x1')
                qt = qkv_range(h0, qkv0_s, 2 * NB + XB, 3 * NB)
            for r0, k in zip(lcs, _spread(len(lcs), 0, L10STOP * len(qt))):
                if r0 >= L10FREE * LC:
                    fence_x(qt[k])
                l1(h1, 1, r0, LC)
            wait('wo')
            perm_wo()
            qkv_s[KO:, 0:HALO, :] = qkv0_s[KO:, TM:TM + HALO, :]
            qt = qkv_range(h1, qkv_s, 0, 2 * NB + QV)
            ks = _spread(nun, A0START * len(qt), A0STOP * len(qt))
            pipelined(nun, A0LAG, lambda u: attn1(qkv0_s, rcs[u], qt[ks[u]] if u >= A0FREE else None),
                      lambda u, lg: attn2(qkv0_s, o_b[UN], rcs[u], True, lg))
            wo_mm(o_b[UN])
            wait('wmb', 'b1')
            if MERGE0:
                wait('w10', 'w20')
            mb = mod_mm(2 * D, 5 * D)
            mod_s[2] = mb[:, 0:D]
            mod_s[3] = mb[:, D:2 * D]
            mod_s[4] = 1.0 + mb[:, 2 * D:3 * D]
            b1_s[...] = jnp.broadcast_to(b1_v[...].astype(F32).reshape(1, F), (8, F)) * GS
            qt = qkv_range(h1, qkv_s, 2 * NB + QV, 3 * NB)
            x1s, ys = l2_units(0, lcs, [qt[k] if u >= L20FREE else None
                                        for u, k in enumerate(_spread(len(lcs), 0, L20STOP * len(qt)))])
            y = jnp.concatenate(ys, axis=0)
            ends = [k * tpc for k in WSPLITS[1:]]
            usable = [u for u in range(int(A1START * ntok), int(A1STOP * ntok)) if not any(0 < e - u <= SEGMARGIN for e in ends)]
            aidx = [usable[k] for k in _spread(nun, 0, len(usable))]
            lidx = _spread(len(lcs), WSPLITS[-1] * tpc, ntok - L12M)
            acc = None
            ua = 0
            ul = 0
            ol = []
            for n, (f0, fc) in enumerate(fcs):
                if n in WSPLITS:
                    k = WSPLITS.index(n)
                    if n == WSPLITS[-1]:
                        if not OLAST:
                            assert ua == nun
                            wo_mm(o_b[0], 1, UN - 1)
                        wait(f'w1{k}', f'w2{k}', 'wmc', 'b2', 'x2')
                        gb = mod_mm(5 * D, 6 * D)
                        mod_s[5] = gb * (0.5 / GS)
                        mod_s[6] = gb * jnp.broadcast_to(b2_v[...].astype(F32).reshape(1, D), (8, D))
                    elif not (MERGE0 and k == 0):
                        wait(f'w1{k}', f'w2{k}')
                part, tk = mlp(y, f0, fc, True)
                acc = part if acc is None else acc + part
                while ua < nun and aidx[ua] // tpc == n:
                    ol.append(attn(qkv_s, o_b[0], rcs[ua], False, tk[aidx[ua] % tpc],
                                   ol[ua - CHAIN1] if (CHAIN1 and ua >= CHAIN1) else None))
                    ua += 1
                while ul < len(lidx) and lidx[ul] // tpc == n:
                    fence_x(tk[lidx[ul] % tpc])
                    l1(h_b[0], 2, lcs[ul], LC)
                    ul += 1
            out(0, jnp.concatenate(x1s, axis=0), acc, 0, TM)
            if OLAST:
                wo_mm(o_b[0], 1, UN - 1)
            ocopy(0, 0, TM, 0).start()

        def head_rows(u):
            if RH == 0:
                return [], []
            return [xh_b[u][...]], [pltpu.bitcast(yh_b[u][...], BF16)]

        def tile(t, u, tnext):
            hcur, hnext, o_s = h_b[u], h_b[(u + 1) % UN], o_b[u]
            qkv_s[KO:, 0:HALO, :] = qkv_s[KO:, TM:TM + HALO, :]
            qt = qkv_part(hcur, qkv_s, 0) + qkv_part(hcur, qkv_s, 1) + qkv_part(hcur, qkv_s, 2)
            x1s, ys = head_rows((u - 1) % UN)
            l2cs = list(range(RH, TM, LC))
            xa, ya = l2_units(t - 1, l2cs, [qt[k] for k in _spread(len(l2cs), L2START * len(qt), L2STOP * len(qt))])
            x1s, ys = x1s + xa, ys + ya
            hl = []
            for r0, k in zip(lcs, _spread(len(lcs), L1START * len(qt), L1STOP * len(qt))):
                fence_x(qt[k])
                hl.append(l1(hnext, tnext, r0, LC))
            y = jnp.concatenate(ys, axis=0)
            aidx = _spread(nun, ASTART * ntok, ASTOP * ntok)
            acc = None
            ua = 0
            base = 0
            ol = []
            for f0, fc in sfcs:
                part, tk = mlp(y, f0, fc)
                acc = part if acc is None else acc + part
                while ua < nun and aidx[ua] < base + len(tk):
                    dep = None
                    if CHAIN and ua >= CHAIN:
                        dep = ol[ua - CHAIN]
                    if L1CHAIN and L1CHAIN <= ua < L1CHAIN + len(hl) // L1PER:
                        k0 = (ua - L1CHAIN) * L1PER
                        dl = hl[k0]
                        for e in hl[k0 + 1:k0 + L1PER]:
                            dl = dl | e
                        dep = dl if dep is None else dep | dl
                    ol.append(attn(qkv_s, o_s, rcs[ua], False, tk[aidx[ua] - base], dep))
                    ua += 1
                base += len(tk)
            assert base == ntok and ua == nun
            out(t - 1, jnp.concatenate(x1s, axis=0), acc, 0, TM)
            wo_mm(o_s, t, u)

        @pl.when(i == 2)
        def _():
            cp('xr').wait()

        @pl.when(jnp.logical_and(i > 1, i < NBLK + 2))
        def _():
            if ONLY in (None, 's'):
              with ns('steady'):
                t0 = 2 + (i - 2) * UN
                for u in range(UN):
                    tn = t0 + u + 1
                    if u == UN - 1:
                        tn = jnp.minimum(tn, NT - 1)
                    tile(t0 + u, u, tn)
                ocopy(t0 - 1, 0, UN * TM, i - 1).start()

        @pl.when(i == NBLK + 2)
        def _():
          if ONLY not in (None, 'e'):
              return
          with ns('epilogue'):
            small = [(sum(EFCS[:k]), EFCS[k]) for k in range(len(EFCS))]
            parts = ([RH] if RH else []) + list(ESPLIT)
            h0 = 0
            tk0 = None
            for e, hm in enumerate(parts):
                if e == 0 and RH:
                    x1s, ys = head_rows(UN - 1)
                else:
                    cs = list(range(h0, h0 + hm, LC))
                    if tk0 is not None and e == 1:
                        tks = [tk0[k] for k in _spread(len(cs), 0, EL2STOP * len(tk0))]
                    else:
                        tks = [None] * len(cs)
                    x1s, ys = l2_units(NT - 1, cs, tks)
                y = jnp.concatenate(ys, axis=0)
                acc = None
                for n, (f0, fc) in enumerate(small if hm < 128 else sfcs):
                    part, tk = mlp(y, f0, fc)
                    if n == 0 and e == 0:
                        tk0 = tk
                    acc = part if acc is None else acc + part
                out(NT - 1, jnp.concatenate(x1s, axis=0), acc, h0, hm)
                if EDMA:
                    ocopy(NT - 1, h0, hm, NBLK + 1 + e).start()
                h0 += hm
            if not EDMA:
                ocopy(NT - 1, 0, TM, NBLK + 1).start()
            ocopy(0, 0, TM, 0).wait()
            for k in range(NBLK):
                ocopy(1 + k * UN, 0, UN * TM, k + 1).wait()
            if EDMA:
                h0 = 0
                for e, hm in enumerate(parts):
                    ocopy(NT - 1, h0, hm, NBLK + 1 + e).wait()
                    h0 += hm
            else:
                ocopy(NT - 1, 0, TM, NBLK + 1).wait()

    def fn(A_x, A_wqkv, A_wo, B_x, B_w1, B_b1, B_w2, B_b2, c, w_mod):
        B, S, D = A_x.shape
        F = B_w1.shape[1]
        NT = S // TM
        assert (NT - 2) % UN == 0
        NBLK = (NT - 2) // UN
        NB = D // 128
        x = A_x.reshape(S, D)
        anyspec = pl.BlockSpec(memory_space=pl.ANY)
        out = pl.pallas_call(
            kernel,
            grid=(NBLK + 3,),
            in_specs=[anyspec] * 9,
            out_specs=anyspec,
            out_shape=jax.ShapeDtypeStruct((S, D), A_x.dtype),
            scratch_shapes=[
                pltpu.VMEM((S + 16, D), BF16),
                pltpu.VMEM((D, 3 * D), BF16),
                pltpu.VMEM((D, D), BF16),
                pltpu.VMEM((D, F), BF16),
                pltpu.VMEM((F,), BF16),
                pltpu.VMEM((F, D), BF16),
                pltpu.VMEM((D,), BF16),
                pltpu.VMEM((1, D), BF16),
                pltpu.VMEM((D, 6 * D), BF16),
                pltpu.VMEM((7, 8, D), F32),
                pltpu.VMEM((8, F), F32),
                pltpu.VMEM((8, D), F32),
                pltpu.VMEM((D // 2, 3 * D), U32),
                pltpu.VMEM((NB, D // 2, 128), U32),
                pltpu.VMEM((D // 2, D), U32),
                pltpu.VMEM((3 * NB, TM + HALO, 128), F32),
                pltpu.VMEM((3 * NB, TM + HALO, 128), F32),
                pltpu.VMEM((TM + 8, D), F32),
                pltpu.VMEM((S, D), BF16),
                pltpu.VMEM((D // 2, F), U32),
                pltpu.VMEM((F // 2, D), U32),
                pltpu.SMEM((1,), I32),
                pltpu.SemaphoreType.DMA((14 + 2 * len(WSPLITS),)),
                pltpu.SemaphoreType.DMA((NBLK + 2 + len(ESPLIT),)),
            ] + [pltpu.VMEM((TM // 2, D), U32)] * (2 * UN + 2)
              + [pltpu.VMEM((max(RH, 16) // 2, D), U32)] * UN
              + [pltpu.VMEM((max(RH, 16), D), F32)] * UN,
            compiler_params=pltpu.CompilerParams(
                dimension_semantics=("arbitrary",),
                vmem_limit_bytes=100 * 1024 * 1024,
            ),
        )(x, A_wqkv, A_wo, B_w1, B_b1, B_w2, B_b2, c, w_mod)
        return out.reshape(B, S, D)
    return fn


pallas_adaLN_cond__sliding_local_dilated__mixer_channel_mlp__prompt_kernel = jax.jit(make_kernel())
```

```python
import jax
import jax.numpy as jnp
from jax import lax
import jax.experimental.pallas as pl
import jax.experimental.pallas.tpu as pltpu

F32 = jnp.float32
BF16 = jnp.bfloat16
U32 = jnp.uint32
I32 = jnp.int32

DH = 16
W = 8
DIL = 2
HALO = 16
EPS = 1e-5
LOG2E = 1.4426950408889634
GC0 = 0.7978845608028654
GS = (GC0 * 0.044715) ** (1.0 / 3.0)
GK = GC0 / GS

TM = 256
UN = 2
RC = 16
LC = 16
RH = 64
FC = 256
SFCS = (512, 512, 512, 256)
WSPLITS = (0, 1, 3, 5)
ESPLIT = (160, 32)
NTOK = 8


def _center(x):
    inv = 1.0 / x.shape[-1]
    m = jnp.sum(x, axis=-1, keepdims=True) * inv
    ms = jnp.sum(x * x, axis=-1, keepdims=True) * inv
    v = jnp.maximum(ms - m * m, 0.0)
    return x - m, lax.rsqrt(v + EPS)


def _spread(n, lo, hi):
    return [int(lo + (u * (hi - lo)) / n) for u in range(n)]


def _rep8(v, n):
    return v if n == 8 else jnp.concatenate([v] * (n // 8), axis=0)


def _pipelined(n, lag, stage1, stage2):
    mid, res = {}, []
    for u in range(n + lag):
        if u < n:
            mid[u] = stage1(u)
        if u >= lag:
            res.append(stage2(u - lag, mid.pop(u - lag)))
    return res


def _kernel(x_hbm, wqkv_hbm, wo_hbm, w1_hbm, b1_hbm, w2_hbm, b2_hbm, c_hbm, wmod_hbm,
            out_hbm,
            x_s, wqkv_v, wo_v, w1_v, b1_v, w2_v, b2_v, c_v, wmod_v,
            mod_s, b1_s, s8_s, wqkv_p, wo_f, wo_p, qkv_s, qkv0_s, a_s, y_s, w1_p, w2_p,
            z_s, sem, osem, *bufs):
    h_b = bufs[:UN + 1]
    o_b = bufs[UN + 1:2 * UN + 2]
    yh_b = bufs[2 * UN + 2:3 * UN + 2]
    xh_b = bufs[3 * UN + 2:4 * UN + 2]
    i = pl.program_id(0)
    S, D = x_hbm.shape
    F = w1_hbm.shape[-1]
    NT = S // TM
    NBLK = (NT - 2) // UN
    NB = D // 128
    QO, KO, VO = 0, NB, 2 * NB
    fcs = [(f0, FC) for f0 in range(0, F, FC)]
    sfcs = [(sum(SFCS[:k]), SFCS[k]) for k in range(len(SFCS))]
    wb = [fcs[k][0] for k in WSPLITS] + [F]
    rcs = list(range(0, TM, RC))
    lcs = list(range(0, TM, LC))
    nun = len(rcs)
    tpc = NTOK * (FC // 128 + FC * D // 65536)
    ntok = tpc * len(fcs)

    srcdst = {}

    def defcopy(name, src, dst):
        srcdst[name] = (src, dst, len(srcdst))

    defcopy('c', c_hbm, c_v)
    defcopy('b1', b1_hbm, b1_v)
    defcopy('b2', b2_hbm, b2_v)
    for p, n in enumerate(('wq', 'wk', 'wv')):
        defcopy(n, wqkv_hbm.at[:, p * D:(p + 1) * D], wqkv_v.at[:, p * D:(p + 1) * D])
    defcopy('wma', wmod_hbm.at[:, 0:2 * D], wmod_v.at[:, 0:2 * D])
    defcopy('wmb', wmod_hbm.at[:, 2 * D:5 * D], wmod_v.at[:, 2 * D:5 * D])
    defcopy('wmc', wmod_hbm.at[:, 5 * D:6 * D], wmod_v.at[:, 5 * D:6 * D])
    defcopy('wo', wo_hbm, wo_v)
    for k in range(len(WSPLITS)):
        defcopy(f'w1{k}', w1_hbm.at[:, wb[k]:wb[k + 1]], w1_v.at[:, wb[k]:wb[k + 1]])
        defcopy(f'w2{k}', w2_hbm.at[wb[k]:wb[k + 1], :], w2_v.at[wb[k]:wb[k + 1], :])
    for t in range(3):
        defcopy(f'x{t}', x_hbm.at[t * TM:(t + 1) * TM, :], x_s.at[t * TM:(t + 1) * TM, :])
    defcopy('xr', x_hbm.at[3 * TM:S, :], x_s.at[3 * TM:S, :])

    def cp(name):
        src, dst, k = srcdst[name]
        return pltpu.make_async_copy(src, dst, sem.at[k])

    def wait(*names):
        for n in names:
            cp(n).wait()

    def rows(t, r0, n):
        if isinstance(t, int):
            return pl.ds(t * TM + r0, n)
        return pl.ds(pl.multiple_of(t * TM + r0, 16), n)

    def ocopy(t, r0, n, k):
        return pltpu.make_async_copy(y_s.at[rows(t, r0, n), :], out_hbm.at[rows(t, r0, n), :], osem.at[k])

    def modv(k, n):
        return _rep8(mod_s[k], n)

    def fence_a(tok):
        a_s[pl.ds(pl.multiple_of(TM + 8 * z_s[0], 8), 8), 0:128] = tok

    def fence_x(tok):
        x_s[pl.ds(pl.multiple_of(S + 16 * z_s[0], 16), 16), 0:128] = (
            jnp.concatenate([tok, tok], axis=0).astype(BF16))

    def tokzero(tok):
        return pltpu.bitcast(tok, I32) & jnp.full((8, 128), z_s[0], I32)

    def tie(v, tz):
        t = _rep8(tz, v.shape[0])
        if v.shape[1] > 128:
            t = jnp.concatenate([t] * (v.shape[1] // 128), axis=1)
        return pltpu.bitcast(pltpu.bitcast(v, I32) | t, v.dtype)

    def toks_of(r, cstep):
        return [r[k:k + 8, c:c + 128] for c in range(0, r.shape[1], cstep)
                for k in range(0, r.shape[0], TM // NTOK)]

    def perm_cols(p):
        lane = lax.broadcasted_iota(I32, (D // 2, 128), 1)
        b = (lane >> 2) & 3
        blk = [pltpu.bitcast(wqkv_v[:, p * D + k * 128:p * D + (k + 1) * 128], U32) for k in range(NB)]
        prev = None
        for j in range(NB):
            m = jnp.where(b == 0, blk[j], blk[(j + 1) % NB])
            m = jnp.where(b == 2, blk[(j + 2) % NB], m)
            m = jnp.where(b == 3, blk[(j + 3) % NB], m)
            if prev is not None:
                m = tie(m, tokzero(prev))
            idx = (((lane >> 1) & 7) * 16 + ((((lane >> 4) & 3) + (NB - j)) & 3) * 4
                   + (lane >> 6) * 2 + (lane & 1))
            r = jnp.take_along_axis(m, idx, axis=1)
            wqkv_p[:, p * D + j * 128:p * D + (j + 1) * 128] = r
            prev = r[D // 2 - 8:D // 2, :]

    def perm_wo():
        for k in range(NB):
            wo_f[k] = pltpu.bitcast(wo_v[:, k * 128:(k + 1) * 128], U32)
        for k in range(NB):
            for j in range(NB):
                for e1 in range(2):
                    for ii in range(4):
                        r = j * 64 + e1 * 32 + ii * 8
                        src = ii * 64 + ((ii - j) % 4) * 2 + e1
                        wo_p[r:r + 8, k * 128:(k + 1) * 128] = wo_f[k, pl.ds(src, 8, stride=8), :]

    def mod_mm(c0, c1):
        return jnp.dot(s8_s[...].astype(BF16), wmod_v[:, c0:c1], preferred_element_type=F32)

    def xrows(t, r0, n):
        return x_s[rows(t, r0, n), :].astype(F32)

    def l1_mod(hbuf, xn, r0, n):
        hv = pltpu.bitcast((xn * modv(1, n) + modv(0, n)).astype(BF16), U32)
        hbuf[r0 // 2:(r0 + n) // 2, :] = hv
        return hv[0:8, D - 128:D]

    def l1(hbuf, t, r0, n):
        xc, rs = _center(xrows(t, r0, n))
        return l1_mod(hbuf, xc * rs, r0, n)

    def qkv_cols(hbuf, buf, j0, j1):
        h = pltpu.bitcast(hbuf[...], BF16)
        r = jnp.dot(h, pltpu.bitcast(wqkv_p[:, j0 * 128:j1 * 128], BF16), preferred_element_type=F32)
        if j0 < NB:
            r = r * ((DH ** -0.5) * LOG2E)
        for j in range(j0, j1):
            buf[j, HALO:HALO + TM, :] = r[:, (j - j0) * 128:(j - j0 + 1) * 128]
        return toks_of(r, 128)

    def qkv_range(hbuf, buf, j0, j1):
        tk = []
        if j0 < NB:
            tk += qkv_cols(hbuf, buf, j0, min(j1, NB))
            j0 = NB
        if j1 > j0:
            tk += qkv_cols(hbuf, buf, j0, j1)
        return tk

    def attn1(buf, r0, tok=None, dep=None):
        q = [buf[QO + j, HALO + r0:HALO + r0 + RC, :] for j in range(NB)]
        if tok is not None:
            tz = tokzero(tok)
            if dep is not None:
                tz = tz | tokzero(dep)
            q = [tie(v, tz) for v in q]
        lg = []
        for w in range(W):
            st = HALO + r0 - DIL * w
            acc = q[0] * buf[KO, st:st + RC, :]
            for j in range(1, NB):
                acc = acc + q[j] * buf[KO + j, st:st + RC, :]
            lg.append(acc)
        rl = [pltpu.roll(a, 64, 1) for a in lg]
        return [a + b for a, b in zip(lg, rl)]

    def attn2(buf, o_s, r0, first, lg):
        swap = lax.broadcasted_iota(I32, (RC, 128), 1) ^ 1
        sw = [jnp.take_along_axis(a, swap, axis=1) for a in lg]
        lg = [a + b for a, b in zip(lg, sw)]
        if first and r0 < HALO:
            row = r0 + lax.broadcasted_iota(I32, (RC, 128), 0)
            lg = [lg[0]] + [jnp.where(row >= DIL * w, lg[w], -1e9 * LOG2E) for w in range(1, W)]
        m = lg[0]
        for w in range(1, W):
            m = jnp.maximum(m, lg[w])
        p = [jnp.exp2(l - m) for l in lg]
        den = p[0]
        for w in range(1, W):
            den = den + p[w]
        rden = pl.reciprocal(den, approx=True)
        for j in range(NB):
            st = HALO + r0
            acc = p[0] * buf[VO + j, st:st + RC, :]
            for w in range(1, W):
                st = HALO + r0 - DIL * w
                acc = acc + p[w] * buf[VO + j, st:st + RC, :]
            ov = pltpu.bitcast((acc * rden).astype(BF16), U32)
            o_s[r0 // 2:(r0 + RC) // 2, j * 128:(j + 1) * 128] = ov
        return ov

    def attn(buf, o_s, r0, tok, dep):
        return attn2(buf, o_s, r0, False, attn1(buf, r0, tok, dep))

    def l2_a(x1, n):
        xc, rs = _center(x1)
        return x1, (xc * rs) * modv(4, n) + modv(3, n)

    def l2_b(h2):
        hc, rs2 = _center(h2)
        return (hc * (rs2 * GS)).astype(BF16)

    def l2_units(t, cs, toks):
        def s1(k):
            if toks[k] is not None:
                fence_a(toks[k])
            r0 = cs[k]
            return l2_a(xrows(t, r0, LC) + modv(2, LC) * a_s[r0:r0 + LC, :], LC)
        res = _pipelined(len(cs), 2, s1, lambda k, m: (m[0], l2_b(m[1])))
        return [r[0] for r in res], [r[1] for r in res]

    def wo_mm(o_s, t=None, u=None):
        wo = pltpu.bitcast(wo_p[...], BF16)
        if t is None:
            a_s[0:TM, :] = jnp.dot(pltpu.bitcast(o_s[...], BF16), wo, preferred_element_type=F32)
            return
        ah = jnp.dot(pltpu.bitcast(o_s[0:RH // 2, :], BF16), wo, preferred_element_type=F32)
        a = jnp.dot(pltpu.bitcast(o_s[RH // 2:TM // 2, :], BF16), wo, preferred_element_type=F32)
        a_s[RH:TM, :] = a
        tk = toks_of(a, 128)
        hcs = list(range(0, RH, LC))
        ks = _spread(len(hcs), 0.1 * len(tk), 0.3 * len(tk))

        def s1(k):
            r0 = hcs[k]
            x1 = xrows(t, r0, LC) + modv(2, LC) * tie(ah[r0:r0 + LC, :], tokzero(tk[ks[k]]))
            xh_b[u][r0:r0 + LC, :] = x1
            return l2_a(x1, LC)[1]

        def s2(k, h2):
            r0 = hcs[k]
            yh_b[u][r0 // 2:(r0 + LC) // 2, :] = pltpu.bitcast(l2_b(h2), U32)
        _pipelined(len(hcs), 2, s1, s2)

    def head_rows(u):
        return [xh_b[u][...]], [pltpu.bitcast(yh_b[u][...], BF16)]

    def mlp(y, f0, fc, raw=False):
        n = y.shape[0]
        if raw:
            w1c = w1_v[:, f0:f0 + fc]
            w2c = w2_v[f0:f0 + fc, :]
            w1_p[:, f0:f0 + fc] = pltpu.bitcast(w1c, U32)
            w2_p[f0 // 2:(f0 + fc) // 2, :] = pltpu.bitcast(w2c, U32)
        else:
            w1c = pltpu.bitcast(w1_p[:, f0:f0 + fc], BF16)
            w2c = pltpu.bitcast(w2_p[f0 // 2:(f0 + fc) // 2, :], BF16)
        z = jnp.dot(y, w1c, preferred_element_type=F32)
        z = z + _rep8(b1_s[:, f0:f0 + fc], n)
        g = (z + z * jnp.tanh(z * (z * z + GK))).astype(BF16)
        part = jnp.dot(g, w2c, preferred_element_type=F32)
        return part, toks_of(z, 128) + toks_of(part, max(128, min(D, 65536 // fc)))

    def out(t, x1, acc, r0, n):
        y_s[rows(t, r0, n), :] = (x1 + (modv(5, n) * acc + modv(6, n))).astype(BF16)

    @pl.when(i == 0)
    def _():
        z_s[0] = 0
        for n in ('x0', 'c', 'wma', 'wq', 'wk', 'wv', 'x1', 'wo', 'b1', 'b2', 'wmb'):
            cp(n).start()
        for k in range(len(WSPLITS)):
            cp(f'w1{k}').start()
            cp(f'w2{k}').start()
        for n in ('wmc', 'x2', 'xr'):
            cp(n).start()
        qkv0_s[KO:, 0:HALO, :] = jnp.zeros((2 * NB, HALO, 128), F32)

    @pl.when(i == 1)
    def _():
        h0, h1 = h_b[UN - 1], h_b[UN]
        wait('x0', 'c')
        c = c_v[...].astype(F32)
        s8_s[...] = jnp.broadcast_to(c * jax.nn.sigmoid(c), (8, D))
        for r0 in lcs:
            xc, rs = _center(xrows(0, r0, LC))
            a_s[r0:r0 + LC, :] = xc * rs
        wait('wma')
        ma = mod_mm(0, 2 * D)
        mod_s[0] = ma[:, 0:D]
        mod_s[1] = 1.0 + ma[:, D:2 * D]
        for r0 in lcs:
            l1_mod(h0, a_s[r0:r0 + LC, :], r0, LC)
        wait('wq')
        perm_cols(0)
        qkv_range(h0, qkv0_s, 0, NB - 1)
        wait('wk')
        perm_cols(1)
        qkv_range(h0, qkv0_s, NB - 1, 2 * NB - 1)
        wait('wv', 'x1')
        perm_cols(2)
        qt = qkv_range(h0, qkv0_s, 2 * NB - 1, 3 * NB)
        for r0, k in zip(lcs, _spread(len(lcs), 0, 0.75 * len(qt))):
            if r0 >= 4 * LC:
                fence_x(qt[k])
            l1(h1, 1, r0, LC)
        wait('wo')
        perm_wo()
        qkv_s[KO:, 0:HALO, :] = qkv0_s[KO:, TM:TM + HALO, :]
        qt = qkv_range(h1, qkv_s, 0, 2 * NB + 1)
        ks = _spread(nun, 0, 0.3 * len(qt))
        _pipelined(nun, 2, lambda u: attn1(qkv0_s, rcs[u], qt[ks[u]] if u >= 4 else None),
                   lambda u, lg: attn2(qkv0_s, o_b[UN], rcs[u], True, lg))
        wo_mm(o_b[UN])
        wait('wmb', 'b1', 'w10', 'w20')
        mb = mod_mm(2 * D, 5 * D)
        mod_s[2] = mb[:, 0:D]
        mod_s[3] = mb[:, D:2 * D]
        mod_s[4] = 1.0 + mb[:, 2 * D:3 * D]
        b1_s[...] = jnp.broadcast_to(b1_v[...].astype(F32).reshape(1, F), (8, F)) * GS
        qt = qkv_range(h1, qkv_s, 2 * NB + 1, 3 * NB)
        x1s, ys = l2_units(0, lcs, [qt[k] for k in _spread(len(lcs), 0, 0.3 * len(qt))])
        y = jnp.concatenate(ys, axis=0)
        ends = [k * tpc for k in WSPLITS[1:]]
        usable = [u for u in range(int(0.02 * ntok), int(0.55 * ntok))
                  if not any(0 < e - u <= 10 for e in ends)]
        aidx = [usable[k] for k in _spread(nun, 0, len(usable))]
        lidx = _spread(len(lcs), WSPLITS[-1] * tpc, ntok - 16)
        acc = None
        ua = 0
        ul = 0
        ol = []
        for n, (f0, fc) in enumerate(fcs):
            if n == WSPLITS[-1]:
                k = len(WSPLITS) - 1
                wo_mm(o_b[0], 1, UN - 1)
                wait(f'w1{k}', f'w2{k}', 'wmc', 'b2', 'x2')
                gb = mod_mm(5 * D, 6 * D)
                mod_s[5] = gb * (0.5 / GS)
                mod_s[6] = gb * jnp.broadcast_to(b2_v[...].astype(F32).reshape(1, D), (8, D))
            elif n in WSPLITS[1:]:
                k = WSPLITS.index(n)
                wait(f'w1{k}', f'w2{k}')
            part, tk = mlp(y, f0, fc, True)
            acc = part if acc is None else acc + part
            while ua < nun and aidx[ua] // tpc == n:
                ol.append(attn(qkv_s, o_b[0], rcs[ua], tk[aidx[ua] % tpc], ol[ua - 2] if ua >= 2 else None))
                ua += 1
            while ul < len(lidx) and lidx[ul] // tpc == n:
                fence_x(tk[lidx[ul] % tpc])
                l1(h_b[0], 2, lcs[ul], LC)
                ul += 1
        out(0, jnp.concatenate(x1s, axis=0), acc, 0, TM)
        ocopy(0, 0, TM, 0).start()

    def tile(t, u, tnext):
        hcur, hnext, o_s = h_b[u], h_b[(u + 1) % UN], o_b[u]
        qkv_s[KO:, 0:HALO, :] = qkv_s[KO:, TM:TM + HALO, :]
        qt = []
        for p in range(3):
            qt += qkv_cols(hcur, qkv_s, p * NB, (p + 1) * NB)
        x1s, ys = head_rows((u - 1) % UN)
        l2cs = list(range(RH, TM, LC))
        xa, ya = l2_units(t - 1, l2cs, [qt[k] for k in _spread(len(l2cs), 0, 0.45 * len(qt))])
        x1s, ys = x1s + xa, ys + ya
        hl = []
        for r0, k in zip(lcs, _spread(len(lcs), 0.5 * len(qt), len(qt))):
            fence_x(qt[k])
            hl.append(l1(hnext, tnext, r0, LC))
        y = jnp.concatenate(ys, axis=0)
        aidx = _spread(nun, 0.03 * ntok, 0.8 * ntok)
        acc = None
        ua = 0
        base = 0
        ol = []
        for f0, fc in sfcs:
            part, tk = mlp(y, f0, fc)
            acc = part if acc is None else acc + part
            while ua < nun and aidx[ua] < base + len(tk):
                dep = ol[ua - 2] if ua >= 2 else None
                if 2 <= ua < 2 + len(hl) // 4:
                    k0 = (ua - 2) * 4
                    dep = dep | (((hl[k0] | hl[k0 + 1]) | hl[k0 + 2]) | hl[k0 + 3])
                ol.append(attn(qkv_s, o_s, rcs[ua], tk[aidx[ua] - base], dep))
                ua += 1
            base += len(tk)
        out(t - 1, jnp.concatenate(x1s, axis=0), acc, 0, TM)
        wo_mm(o_s, t, u)

    @pl.when(i == 2)
    def _():
        cp('xr').wait()

    @pl.when(jnp.logical_and(i > 1, i < NBLK + 2))
    def _():
        t0 = 2 + (i - 2) * UN
        for u in range(UN):
            tn = t0 + u + 1
            if u == UN - 1:
                tn = jnp.minimum(tn, NT - 1)
            tile(t0 + u, u, tn)
        ocopy(t0 - 1, 0, UN * TM, i - 1).start()

    @pl.when(i == NBLK + 2)
    def _():
        parts = [RH] + list(ESPLIT)
        h0 = 0
        tk0 = None
        for e, hm in enumerate(parts):
            if e == 0:
                x1s, ys = head_rows(UN - 1)
            else:
                cs = list(range(h0, h0 + hm, LC))
                if e == 1:
                    tks = [tk0[k] for k in _spread(len(cs), 0, 0.9 * len(tk0))]
                else:
                    tks = [None] * len(cs)
                x1s, ys = l2_units(NT - 1, cs, tks)
            y = jnp.concatenate(ys, axis=0)
            acc = None
            for f0, fc in ([(0, F)] if hm < 128 else sfcs):
                part, tk = mlp(y, f0, fc)
                if e == 0:
                    tk0 = tk
                acc = part if acc is None else acc + part
            out(NT - 1, jnp.concatenate(x1s, axis=0), acc, h0, hm)
            ocopy(NT - 1, h0, hm, NBLK + 1 + e).start()
            h0 += hm
        ocopy(0, 0, TM, 0).wait()
        for k in range(NBLK):
            ocopy(1 + k * UN, 0, UN * TM, k + 1).wait()
        h0 = 0
        for e, hm in enumerate(parts):
            ocopy(NT - 1, h0, hm, NBLK + 1 + e).wait()
            h0 += hm


@jax.jit
def pallas_adaLN_cond__sliding_local_dilated__mixer_channel_mlp__prompt_kernel(
    A_x: jax.Array,
    A_wqkv: jax.Array,
    A_wo: jax.Array,
    B_x: jax.Array,
    B_w1: jax.Array,
    B_b1: jax.Array,
    B_w2: jax.Array,
    B_b2: jax.Array,
    c: jax.Array,
    w_mod: jax.Array,
):
    B, S, D = A_x.shape
    F = B_w1.shape[1]
    NT = S // TM
    NBLK = (NT - 2) // UN
    NB = D // 128
    assert B == 1 and D == 512 and S == (2 + NBLK * UN) * TM and F == sum(SFCS) and F % FC == 0
    anyspec = pl.BlockSpec(memory_space=pl.ANY)
    out = pl.pallas_call(
        _kernel,
        grid=(NBLK + 3,),
        in_specs=[anyspec] * 9,
        out_specs=anyspec,
        out_shape=jax.ShapeDtypeStruct((S, D), A_x.dtype),
        scratch_shapes=[
            pltpu.VMEM((S + 16, D), BF16),
            pltpu.VMEM((D, 3 * D), BF16),
            pltpu.VMEM((D, D), BF16),
            pltpu.VMEM((D, F), BF16),
            pltpu.VMEM((F,), BF16),
            pltpu.VMEM((F, D), BF16),
            pltpu.VMEM((D,), BF16),
            pltpu.VMEM((1, D), BF16),
            pltpu.VMEM((D, 6 * D), BF16),
            pltpu.VMEM((7, 8, D), F32),
            pltpu.VMEM((8, F), F32),
            pltpu.VMEM((8, D), F32),
            pltpu.VMEM((D // 2, 3 * D), U32),
            pltpu.VMEM((NB, D // 2, 128), U32),
            pltpu.VMEM((D // 2, D), U32),
            pltpu.VMEM((3 * NB, TM + HALO, 128), F32),
            pltpu.VMEM((3 * NB, TM + HALO, 128), F32),
            pltpu.VMEM((TM + 8, D), F32),
            pltpu.VMEM((S, D), BF16),
            pltpu.VMEM((D // 2, F), U32),
            pltpu.VMEM((F // 2, D), U32),
            pltpu.SMEM((1,), I32),
            pltpu.SemaphoreType.DMA((14 + 2 * len(WSPLITS),)),
            pltpu.SemaphoreType.DMA((NBLK + 2 + len(ESPLIT),)),
        ] + [pltpu.VMEM((TM // 2, D), U32)] * (2 * UN + 2)
          + [pltpu.VMEM((RH // 2, D), U32)] * UN
          + [pltpu.VMEM((RH, D), F32)] * UN,
        compiler_params=pltpu.CompilerParams(
            dimension_semantics=("arbitrary",),
            vmem_limit_bytes=100 * 1024 * 1024,
        ),
    )(A_x.reshape(S, D), A_wqkv, A_wo, B_w1, B_b1, B_w2, B_b2, c, w_mod)
    return out.reshape(B, S, D)
```
